```python
import os as _os
_os.environ.setdefault("JAX_PLATFORMS", "cpu")
import jax
import jax.numpy as jnp

def _softmax(x, axis=-1):
    return jax.nn.softmax(x, axis=axis)
def _gelu(x):
    return jax.nn.gelu(x, approximate=True)
def _silu(x):
    return jax.nn.silu(x)
def _sigmoid(x):
    return jax.nn.sigmoid(x)
def _layernorm(x, axis=-1, eps=1e-5):
    m = jnp.mean(x, axis=axis, keepdims=True)
    v = jnp.var(x, axis=axis, keepdims=True)
    return (x - m) / jnp.sqrt(v + eps)
def _scatter_add(tgt, idx, src, axis=0):
    return tgt.at[idx].add(src)
def _segment_sum(src, seg, n):
    return jax.ops.segment_sum(src, seg, n)
class _Rng:
    def __init__(self, key):
        self._k = key
    def _next(self):
        self._k, sub = jax.random.split(self._k)
        return sub
    def normal(self, shape):
        return jax.random.normal(self._next(), shape, dtype=jnp.bfloat16)
    def randint(self, lo, hi, shape):
        return jax.random.randint(self._next(), shape, lo, hi, dtype=jnp.int32)
    def uniform(self, shape, lo=0.0, hi=1.0):
        return jax.random.uniform(self._next(), shape, jnp.bfloat16, lo, hi)
    def permutation(self, n):
        return jax.random.permutation(self._next(), n)


kernel_name = 'sequential_preLN__linear_kernel_hedgehog__dense_activation_squared_relu__prompt'

def setup_inputs():
    _rng = _Rng(jax.random.key(int.from_bytes(__import__("os").urandom(4), "little")))
    _w = (lambda a: (lambda t: t.astype(jnp.bfloat16) if jnp.issubdtype(t.dtype, jnp.floating) else t)(jnp.asarray(a)))
    def _A_setup():
        B, S, D, H = 1, 2048, 512, 32
        Dh = D // H
        return {
            "x": _w((lambda *s: _rng.normal(s) * 0.05)(B, S, D)),
            "wqkv": _w((lambda *s: _rng.normal(s) * 0.2)(D, 3 * D)),
            "w_phi": _w((lambda *s: _rng.normal(s) * 0.2)(H, Dh, Dh) * (Dh ** -0.5)),
            "wo": _w((lambda *s: _rng.normal(s) * 0.05)(D, D)),
        }
    _A_in = _A_setup()

    def _B_setup():
        B, S, D, F = 1, 2048, 512, 1792
        return {
            "x": _w((lambda *s: _rng.normal(s) * 0.05)(B, S, D)),
            "w1": _w((lambda *s: _rng.normal(s) * 0.05)(D, F)),
            "b1": _w((lambda *s: _rng.normal(s) * 0.05)(F)),
            "w2": _w((lambda *s: _rng.normal(s) * 0.05)(F, D)),
            "b2": _w((lambda *s: _rng.normal(s) * 0.05)(D)),
        }
    _B_in = _B_setup()

    return {
        "A_x": _A_in["x"],
        "A_wqkv": _A_in["wqkv"],
        "A_w_phi": _A_in["w_phi"],
        "A_wo": _A_in["wo"],
        "B_x": _B_in["x"],
        "B_w1": _B_in["w1"],
        "B_b1": _B_in["b1"],
        "B_w2": _B_in["w2"],
        "B_b2": _B_in["b2"],
    }

def reference(A_x, A_wqkv, A_w_phi, A_wo, B_x, B_w1, B_b1, B_w2, B_b2):
    def _A_ref(x, wqkv, w_phi, wo):
        B, S, D = x.shape
        H = 32; Dh = D // H
        qkv = (lambda x, *d: x.transpose(*d))((x @ wqkv).reshape(B, S, 3, H, Dh), 2, 0, 3, 1, 4)
        q, k, v = qkv[0], qkv[1], qkv[2]
        pq = jnp.einsum("bhsd,hdf->bhsf", q, w_phi)
        pk = jnp.einsum("bhsd,hdf->bhsf", k, w_phi)
        phi_q = jnp.concatenate([_softmax(pq, axis=-1), _softmax(-pq, axis=-1)], axis=-1)
        phi_k = jnp.concatenate([_softmax(pk, axis=-1), _softmax(-pk, axis=-1)], axis=-1)
        kv = jnp.einsum("bhsf,bhsd->bhfd", phi_k, v)
        z  = jnp.einsum("bhsf->bhf", phi_k)
        num = jnp.einsum("bhqf,bhfd->bhqd", phi_q, kv)
        den = jnp.einsum("bhqf,bhf->bhq", phi_q, z)[..., None] + 1e-6
        o = num / den
        return (lambda x, *d: x.transpose(*d))(o, 0, 2, 1, 3).reshape(B, S, D) @ wo

    def _B_ref(x, w1, b1, w2, b2):
        h = jnp.einsum("bsd,df->bsf", x, w1) + b1
        zero = jnp.zeros_like(h)
        r = jnp.where(h > zero, h, zero)
        h = r * r
        out = jnp.einsum("bsf,fd->bsd", h, w2) + b2
        return out

    x = A_x
    h = x + _A_ref(_layernorm(x, axis=-1), A_wqkv, A_w_phi, A_wo)
    h2 = h + _B_ref(_layernorm(h, axis=-1), B_w1, B_b1, B_w2, B_b2)
    return h2
```

```python
import functools

import jax
import jax.numpy as jnp
import jax.experimental.pallas as pl
import jax.experimental.pallas.tpu as pltpu
from jax import lax

S, D, H, DH, F = 2048, 512, 32, 16, 1792
G = D // 128
T = 256
NT = S // T
FC = 256
LN_EPS = 1e-5
DEN_EPS = 1e-6

_NT_DIMS = (((1,), (1,)), ((), ()))
bf16 = jnp.bfloat16
f32 = jnp.float32


def _dot(a, b):
    return jnp.dot(a, b, preferred_element_type=f32)


def _dot_nt(a, b):
    return lax.dot_general(a, b, _NT_DIMS, preferred_element_type=f32)


def _layernorm(x):
    m = jnp.mean(x, axis=-1, keepdims=True)
    xc = x - m
    v = jnp.mean(xc * xc, axis=-1, keepdims=True)
    return xc * lax.rsqrt(v + LN_EPS)


def _kernel(x_ref, wqkv_ref, wphi_ref, b1_ref, b2_ref, wo_hbm, w1_hbm, w2_hbm,
            o_ref,
            wqkT_s, wo_s, wop_s, w1_s, w2_s, phiq_s, kv_s, z_s, kvT_s, sems):
    i = pl.program_id(0)

    def weight_copies():
        return (
            pltpu.make_async_copy(wo_hbm, wo_s, sems.at[0]),
            pltpu.make_async_copy(w1_hbm, w1_s, sems.at[1]),
            pltpu.make_async_copy(w2_hbm, w2_s, sems.at[2]),
        )

    r128 = lax.broadcasted_iota(jnp.int32, (128, 128), 0)
    c128 = lax.broadcasted_iota(jnp.int32, (128, 128), 1)

    @pl.when(i == 0)
    def _():
        for c in weight_copies():
            c.start()
        m = wphi_ref[...].reshape(H * DH, DH)
        er = lax.broadcasted_iota(jnp.int32, (128, DH), 0)
        ec = lax.broadcasted_iota(jnp.int32, (128, DH), 1)
        eT = jnp.where(er // 8 == ec, 1.0, 0.0).astype(bf16)
        pmask = (r128 % 8) == (c128 // 16)
        for g in range(G):
            p = _dot_nt(eT, m[g * 128:(g + 1) * 128, :])
            p = jnp.where(pmask, p, 0.0).astype(bf16)
            for qk in range(2):
                w = wqkv_ref[:, qk * D + g * 128: qk * D + (g + 1) * 128]
                wqkT_s[qk * D + g * 128: qk * D + (g + 1) * 128, :] = (
                    _dot_nt(p, w).astype(bf16))
        kv_s[...] = jnp.zeros(kv_s.shape, f32)
        z_s[...] = jnp.zeros(z_s.shape, f32)

    @pl.when(i < NT)
    def _():
        xn = _layernorm(x_ref[...].astype(f32)).astype(bf16)
        pT = _dot_nt(wqkT_s[...], xn)
        v = _dot(xn, wqkv_ref[:, 2 * D:3 * D]).astype(bf16)
        for qk in range(2):
            for g in range(G):
                r0 = qk * D + g * 128
                p = pT[r0:r0 + 128, :].reshape(DH, 8, T)
                mx = jnp.max(p, axis=0, keepdims=True)
                mn = jnp.min(p, axis=0, keepdims=True)
                ep = jnp.exp(p - mx)
                en = jnp.exp(mn - p)
                sp = jnp.sum(ep, axis=0, keepdims=True)
                sn = jnp.sum(en, axis=0, keepdims=True)
                pp = (ep * (1.0 / sp)).reshape(128, T)
                pn = (en * (1.0 / sn)).reshape(128, T)
                phi = jnp.concatenate([pp, pn], axis=0)
                phib = phi.astype(bf16)
                if qk == 0:
                    phiq_s[i, g * 256:(g + 1) * 256, :] = phib
                else:
                    kv_s[g] += _dot(phib, v[:, g * 128:(g + 1) * 128])
                    zz = phi[:, 0:128]
                    for c in range(1, T // 128):
                        zz = zz + phi[:, c * 128:(c + 1) * 128]
                    z_s[g] += zz

    @pl.when(i == NT)
    def _():
        for c in weight_copies():
            c.wait()
        permT = jnp.where((r128 // 8 == c128 % 16) & (r128 % 8 == c128 // 16),
                          1.0, 0.0).astype(bf16)
        r2 = lax.broadcasted_iota(jnp.int32, (128, 256), 0)
        c2 = lax.broadcasted_iota(jnp.int32, (128, 256), 1)
        kmask = (r2 % 8) == (c2 % 8)
        r3 = lax.broadcasted_iota(jnp.int32, (16, 256), 0)
        c3 = lax.broadcasted_iota(jnp.int32, (16, 256), 1)
        zmask = r3 == (c3 % 8)
        ones = jnp.ones((16, 128), f32)
        for g in range(G):
            kvT = _dot_nt(permT, kv_s[g].astype(bf16))
            kvT_s[g, 0:128, :] = jnp.where(kmask, kvT, 0.0).astype(bf16)
            zrow = lax.dot_general(ones, z_s[g], _NT_DIMS,
                                   preferred_element_type=f32,
                                   precision=lax.Precision.HIGHEST)
            kvT_s[g, 128:144, :] = jnp.where(zmask, zrow, 0.0).astype(bf16)
            wop_s[g * 128:(g + 1) * 128, :] = _dot(
                permT, wo_s[g * 128:(g + 1) * 128, :]).astype(bf16)

    @pl.when(i >= NT)
    def _():
        t = i - NT
        x = x_ref[...].astype(f32)
        oTs = []
        for g in range(G):
            nd = _dot(kvT_s[g], phiq_s[t, g * 256:(g + 1) * 256, :])
            den = nd[128:136, :] + DEN_EPS
            num = nd[0:128, :].reshape(DH, 8, T)
            oTs.append((num * (1.0 / den)[None]).reshape(128, T))
        oT = jnp.concatenate(oTs, axis=0)
        o = oT.T.astype(bf16)
        h = x + _dot(o, wop_s[...])
        hn = _layernorm(h).astype(bf16)
        acc = h + b2_ref[...].astype(f32)
        for c in range(F // FC):
            h1 = _dot(hn, w1_s[:, c * FC:(c + 1) * FC])
            h1 = h1 + b1_ref[:, c * FC:(c + 1) * FC].astype(f32)
            h1 = jnp.maximum(h1, 0.0)
            h1 = (h1 * h1).astype(bf16)
            acc = acc + _dot(h1, w2_s[c * FC:(c + 1) * FC, :])
        o_ref[...] = acc.astype(o_ref.dtype)


@jax.jit
def pallas_sequential_preLN__linear_kernel_hedgehog__dense_activation_squared_relu__prompt_kernel(
    A_x: jax.Array,
    A_wqkv: jax.Array,
    A_w_phi: jax.Array,
    A_wo: jax.Array,
    B_x: jax.Array,
    B_w1: jax.Array,
    B_b1: jax.Array,
    B_w2: jax.Array,
    B_b2: jax.Array,
):
    del B_x
    b1 = B_b1.reshape(1, F)
    b2 = B_b2.reshape(1, D)

    grid_spec = pltpu.PrefetchScalarGridSpec(
        num_scalar_prefetch=0,
        grid=(2 * NT,),
        in_specs=[
            pl.BlockSpec((None, T, D), lambda i: (0, i % NT, 0)),
            pl.BlockSpec((D, 3 * D), lambda i: (0, 0)),
            pl.BlockSpec((H, DH, DH), lambda i: (0, 0, 0)),
            pl.BlockSpec((1, F), lambda i: (0, 0)),
            pl.BlockSpec((1, D), lambda i: (0, 0)),
            pl.BlockSpec(memory_space=pl.ANY),
            pl.BlockSpec(memory_space=pl.ANY),
            pl.BlockSpec(memory_space=pl.ANY),
        ],
        out_specs=pl.BlockSpec((None, T, D), lambda i: (0, jnp.maximum(i - NT, 0), 0)),
        scratch_shapes=[
            pltpu.VMEM((2 * D, D), bf16),
            pltpu.VMEM((D, D), bf16),
            pltpu.VMEM((D, D), bf16),
            pltpu.VMEM((D, F), bf16),
            pltpu.VMEM((F, D), bf16),
            pltpu.VMEM((NT, 2 * D, T), bf16),
            pltpu.VMEM((G, 256, 128), f32),
            pltpu.VMEM((G, 256, 128), f32),
            pltpu.VMEM((G, 144, 256), bf16),
            pltpu.SemaphoreType.DMA((3,)),
        ],
    )
    return pl.pallas_call(
        _kernel,
        grid_spec=grid_spec,
        out_shape=jax.ShapeDtypeStruct((1, S, D), bf16),
        compiler_params=pltpu.CompilerParams(
            dimension_semantics=("arbitrary",),
            vmem_limit_bytes=100 * 1024 * 1024,
        ),
    )(A_x, A_wqkv, A_w_phi, b1, b2, A_wo, B_w1, B_w2)
```

```python
import jax
import jax.numpy as jnp
import jax.experimental.pallas as pl
import jax.experimental.pallas.tpu as pltpu
from jax import lax

S, D, H, DH, F = 2048, 512, 32, 16, 1792
G = D // 128
TS1 = 256
NXC = S // TS1
N1 = NXC // 2
TS2 = 512
NS2 = 2
N2 = S // (TS2 * NS2)
TO = 256
NOC = S // TO
FC = 256
LN_EPS = 1e-5
DEN_EPS = 1e-6

_NT_DIMS = (((1,), (1,)), ((), ()))
bf16 = jnp.bfloat16
f32 = jnp.float32

_S_WPHI, _S_WQ, _S_WK, _S_WV, _S_WO, _S_W1, _S_W2, _S_B1, _S_B2 = range(9)
_S_X = 9
_S_O = _S_X + NXC
_NSEM = _S_O + NOC


def _dot(a, b):
    return jnp.dot(a, b, preferred_element_type=f32)


def _dot_nt(a, b):
    return lax.dot_general(a, b, _NT_DIMS, preferred_element_type=f32)


def _layernorm(x):
    m = jnp.mean(x, axis=-1, keepdims=True)
    xc = x - m
    v = jnp.mean(xc * xc, axis=-1, keepdims=True)
    return xc * lax.rsqrt(v + LN_EPS)


def _iota(shape, dim):
    return lax.broadcasted_iota(jnp.int32, shape, dim)


def _aligned(c, n):
    return c * n if isinstance(c, int) else pl.multiple_of(c * n, n)


def _kernel(x_hbm, wqkv_hbm, wphi_hbm, b1_hbm, b2_hbm, wo_hbm, w1_hbm, w2_hbm,
            o_hbm,
            x_s, wqkv_s, wphi_s, b1_s, b2_s, wqkT_s, wo_s, w1_s, w2_s,
            xn_s, phiq_s, kv_s, z_s, kvT_s, out_s, sems):

    def cp(src, dst, k):
        return pltpu.make_async_copy(src, dst, sems.at[k])

    def x_copy(c):
        start = _aligned(c, TS1)
        return cp(x_hbm.at[0, pl.ds(start, TS1), :], x_s.at[pl.ds(start, TS1), :], _S_X + c)

    def o_copy(c):
        start = _aligned(c, TO)
        return cp(out_s.at[pl.ds(start, TO), :], o_hbm.at[0, pl.ds(start, TO), :], _S_O + c)

    c_wphi = cp(wphi_hbm, wphi_s, _S_WPHI)
    c_wq = cp(wqkv_hbm.at[:, pl.ds(0, D)], wqkv_s.at[:, pl.ds(0, D)], _S_WQ)
    c_wk = cp(wqkv_hbm.at[:, pl.ds(D, D)], wqkv_s.at[:, pl.ds(D, D)], _S_WK)
    c_wv = cp(wqkv_hbm.at[:, pl.ds(2 * D, D)], wqkv_s.at[:, pl.ds(2 * D, D)], _S_WV)
    c_wo = cp(wo_hbm, wo_s, _S_WO)
    c_w1 = cp(w1_hbm, w1_s, _S_W1)
    c_w2 = cp(w2_hbm, w2_s, _S_W2)
    c_b1 = cp(b1_hbm, b1_s, _S_B1)
    c_b2 = cp(b2_hbm, b2_s, _S_B2)

    def ln_rows(j):
        return _layernorm(x_s[pl.ds(_aligned(j, TS1), TS1), :].astype(f32)).astype(bf16)

    def softmax_group(pT, r0):
        p = pT[r0:r0 + 128, :].reshape(DH, 8, TS1)
        mx = jnp.max(p, axis=0, keepdims=True)
        mn = jnp.min(p, axis=0, keepdims=True)
        ep = jnp.exp(p - mx)
        en = jnp.exp(mn - p)
        sp = jnp.sum(ep, axis=0, keepdims=True)
        sn = jnp.sum(en, axis=0, keepdims=True)
        pp = (ep * (1.0 / sp)).reshape(128, TS1)
        pn = (en * (1.0 / sn)).reshape(128, TS1)
        return jnp.concatenate([pp, pn], axis=0)

    def feat_q(j, pTq):
        for g in range(G):
            phi = softmax_group(pTq, g * 128)
            phiq_s[g * 256:(g + 1) * 256, pl.ds(_aligned(j, TS1), TS1)] = phi.astype(bf16)

    def feat_k(pTk, xn, init=False):
        v = _dot(xn, wqkv_s[:, 2 * D:3 * D]).astype(bf16)
        for g in range(G):
            phi = softmax_group(pTk, g * 128)
            kv = _dot(phi.astype(bf16), v[:, g * 128:(g + 1) * 128])
            zz = phi[:, 0:128]
            for c in range(1, TS1 // 128):
                zz = zz + phi[:, c * 128:(c + 1) * 128]
            if init:
                kv_s[g] = kv
                z_s[g] = zz
            else:
                kv_s[g] += kv
                z_s[g] += zz

    def subtile(j, xn):
        pT = _dot_nt(wqkT_s[...], xn)
        feat_q(j, pT[0:D])
        feat_k(pT[D:2 * D], xn)

    c_wphi.start()
    x_copy(0).start()
    c_wq.start()
    c_wk.start()
    x_copy(1).start()

    c_wphi.wait()
    a = wphi_s[...].reshape(DH * DH, H)
    sel = jnp.where(_iota((H, D), 0) == _iota((H, D), 1) // DH, 1.0, 0.0).astype(bf16)
    b = _dot(a, sel)
    b = jnp.where(_iota((256, D), 0) // DH == _iota((256, D), 1) % DH, b, 0.0).astype(bf16)
    r = jnp.where(_iota((128, 256), 0) // 8 == _iota((128, 256), 1) % DH, 1.0, 0.0).astype(bf16)
    p = _dot(r, b)
    p = jnp.where(_iota((128, D), 0) % 8 == (_iota((128, D), 1) // DH) % 8, p, 0.0).astype(bf16)

    x_copy(0).wait()
    xn0 = ln_rows(0)

    def fold(qk):
        ws = []
        for g in range(G):
            c = qk * G + g
            w = wqkv_s[:, c * 128:(c + 1) * 128]
            ws.append(_dot_nt(p[:, g * 128:(g + 1) * 128], w).astype(bf16))
        wh = jnp.concatenate(ws, axis=0)
        wqkT_s[qk * D:(qk + 1) * D, :] = wh
        return wh

    c_wq.wait()
    c_wv.start()
    pTq0 = _dot_nt(fold(0), xn0)
    c_wk.wait()
    x_copy(1).wait()
    x_copy(2).start()
    pTk0 = _dot_nt(fold(1), xn0)
    feat_q(0, pTq0)
    xn1 = ln_rows(1)

    c_wv.wait()
    x_copy(2).wait()
    for c in range(3, NXC):
        x_copy(c).start()
    c_wo.start()
    c_b1.start()
    c_b2.start()
    c_w1.start()
    c_w2.start()
    feat_k(pTk0, xn0, init=True)
    subtile(1, xn1)
    xn_s[...] = ln_rows(2)

    def phase1(k, carry):
        x_copy(2 * k + 1).wait()

        @pl.when(2 * k + 2 < NXC)
        def _():
            x_copy(2 * k + 2).wait()

        xna = xn_s[...]
        xnb = ln_rows(2 * k + 1)
        subtile(2 * k, xna)
        subtile(2 * k + 1, xnb)
        xn_s[...] = ln_rows(jnp.minimum(2 * k + 2, NXC - 1))
        return carry

    lax.fori_loop(1, N1, phase1, 0)

    c_wo.wait()
    c_b1.wait()
    c_b2.wait()
    c_w1.wait()
    c_w2.wait()
    eye = jnp.where(_iota((128, 128), 0) == _iota((128, 128), 1), 1.0, 0.0).astype(bf16)
    kmask = (_iota((128, 256), 0) // DH) == (_iota((128, 256), 1) % 8)
    zmask = _iota((16, 256), 0) == (_iota((16, 256), 1) % 8)
    ones = jnp.ones((16, 128), bf16)
    for g in range(G):
        kvT = _dot_nt(eye, kv_s[g].astype(bf16))
        kvT_s[g, 0:128, :] = jnp.where(kmask, kvT, 0.0).astype(bf16)
        z = z_s[g]
        zhi = z.astype(bf16)
        zlo = (z - zhi.astype(f32)).astype(bf16)
        zrow = _dot_nt(ones, zhi) + _dot_nt(ones, zlo)
        kvT_s[g, 128:144, :] = jnp.where(zmask, zrow, 0.0).astype(bf16)

    def phase2(t, carry):
        b1 = b1_s[...].reshape(1, F).astype(f32)
        b2 = b2_s[...].reshape(1, D).astype(f32)
        hs = []
        hns = []
        for s in range(NS2):
            rows = pl.ds(_aligned(t * NS2 + s, TS2), TS2)
            x = x_s[rows, :].astype(f32)
            oTs = []
            for g in range(G):
                nd = _dot(kvT_s[g], phiq_s[g * 256:(g + 1) * 256, rows])
                rcp = 1.0 / (nd[128:136, :] + DEN_EPS)
                for j in range(8):
                    oTs.append(nd[j * DH:(j + 1) * DH, :] * rcp[j:j + 1, :])
            oT = jnp.concatenate(oTs, axis=0)
            o = oT.T.astype(bf16)
            h = x + _dot(o, wo_s[...])
            hs.append(h)
            hns.append(_layernorm(h).astype(bf16))
        nc = F // FC
        npc = TS2 // TO
        for s in range(NS2):
            hn = hns[s]
            acc = hs[s] + b2
            for c in range(nc):
                h1 = _dot(hn, w1_s[:, c * FC:(c + 1) * FC])
                h1 = h1 + b1[:, c * FC:(c + 1) * FC]
                h1 = jnp.maximum(h1, 0.0)
                h1 = (h1 * h1).astype(bf16)
                if c < nc - 1:
                    acc = acc + _dot(h1, w2_s[c * FC:(c + 1) * FC, :])
                else:
                    for u in range(npc):
                        oc = (t * NS2 + s) * npc + u
                        part = acc[u * TO:(u + 1) * TO, :] + _dot(
                            h1[u * TO:(u + 1) * TO, :], w2_s[c * FC:(c + 1) * FC, :])
                        out_s[pl.ds(_aligned(oc, TO), TO), :] = part.astype(bf16)
                        o_copy(oc).start()
        return carry

    lax.fori_loop(0, N2, phase2, 0)

    for c in range(NOC):
        o_copy(c).wait()


@jax.jit
def pallas_sequential_preLN__linear_kernel_hedgehog__dense_activation_squared_relu__prompt_kernel(
    A_x: jax.Array,
    A_wqkv: jax.Array,
    A_w_phi: jax.Array,
    A_wo: jax.Array,
    B_x: jax.Array,
    B_w1: jax.Array,
    B_b1: jax.Array,
    B_w2: jax.Array,
    B_b2: jax.Array,
):
    del B_x
    wphi_t = A_w_phi.transpose(1, 2, 0)

    any_spec = pl.BlockSpec(memory_space=pl.ANY)
    return pl.pallas_call(
        _kernel,
        in_specs=[any_spec] * 8,
        out_specs=any_spec,
        scratch_shapes=[
            pltpu.VMEM((S, D), bf16),
            pltpu.VMEM((D, 3 * D), bf16),
            pltpu.VMEM((DH, DH, H), bf16),
            pltpu.VMEM((F,), bf16),
            pltpu.VMEM((D,), bf16),
            pltpu.VMEM((2 * D, D), bf16),
            pltpu.VMEM((D, D), bf16),
            pltpu.VMEM((D, F), bf16),
            pltpu.VMEM((F, D), bf16),
            pltpu.VMEM((TS1, D), bf16),
            pltpu.VMEM((2 * D, S), bf16),
            pltpu.VMEM((G, 256, 128), f32),
            pltpu.VMEM((G, 256, 128), f32),
            pltpu.VMEM((G, 144, 256), bf16),
            pltpu.VMEM((S, D), bf16),
            pltpu.SemaphoreType.DMA((_NSEM,)),
        ],
        out_shape=jax.ShapeDtypeStruct((1, S, D), bf16),
        compiler_params=pltpu.CompilerParams(
            vmem_limit_bytes=100 * 1024 * 1024,
        ),
    )(A_x, A_wqkv, wphi_t, B_b1, B_b2, A_wo, B_w1, B_w2)
```

```python
import jax
import jax.numpy as jnp
import jax.experimental.pallas as pl
import jax.experimental.pallas.tpu as pltpu
from jax import lax

S, D, H, DH, F = 2048, 512, 32, 16, 1792
G = D // 128
TS1 = 256
NXC = S // TS1
NSI = 3
NIT = (NXC - 2) // NSI
TS2 = 512
NS2 = 2
N2 = S // (TS2 * NS2)
TO = 256
NOC = S // TO
NCS = 2
CW = D // NCS
FC = 896
LN_EPS = 1e-5
DEN_EPS = 1e-6

_NT_DIMS = (((1,), (1,)), ((), ()))
bf16 = jnp.bfloat16
f32 = jnp.float32

_S_WPHI, _S_WQ, _S_WK, _S_WV, _S_WO, _S_W1, _S_W2, _S_B1, _S_B2 = range(9)
_S_X = 9
_S_O = _S_X + NXC
_NSEM = _S_O + NOC * NCS


def _dot(a, b):
    return jnp.dot(a, b, preferred_element_type=f32)


def _dot_nt(a, b):
    return lax.dot_general(a, b, _NT_DIMS, preferred_element_type=f32)


def _layernorm(x):
    m = jnp.mean(x, axis=-1, keepdims=True)
    xc = x - m
    v = jnp.mean(xc * xc, axis=-1, keepdims=True)
    return xc * lax.rsqrt(v + LN_EPS)


def _iota(shape, dim):
    return lax.broadcasted_iota(jnp.int32, shape, dim)


def _aligned(c, n):
    return c * n if isinstance(c, int) else pl.multiple_of(c * n, n)


def _kernel(x_hbm, wqkv_hbm, wphi_hbm, b1_hbm, b2_hbm, wo_hbm, w1_hbm, w2_hbm,
            o_hbm,
            x_s, wqkv_s, wphi_s, b1_s, b2_s, wqkT_s, wo_s, w1_s, w2_s,
            xn_s, phiq_s, kv_s, z_s, kvT_s, out_s, sems):

    def cp(src, dst, k):
        return pltpu.make_async_copy(src, dst, sems.at[k])

    def x_copy(c):
        start = _aligned(c, TS1)
        return cp(x_hbm.at[0, pl.ds(start, TS1), :], x_s.at[pl.ds(start, TS1), :], _S_X + c)

    def o_copy(c, w):
        start = _aligned(c, TO)
        return cp(out_s.at[pl.ds(start, TO), pl.ds(w * CW, CW)],
                  o_hbm.at[0, pl.ds(start, TO), pl.ds(w * CW, CW)], _S_O + c * NCS + w)

    c_wphi = cp(wphi_hbm, wphi_s, _S_WPHI)
    c_wq = cp(wqkv_hbm.at[:, pl.ds(0, D)], wqkv_s.at[:, pl.ds(0, D)], _S_WQ)
    c_wk = cp(wqkv_hbm.at[:, pl.ds(D, D)], wqkv_s.at[:, pl.ds(D, D)], _S_WK)
    c_wv = cp(wqkv_hbm.at[:, pl.ds(2 * D, D)], wqkv_s.at[:, pl.ds(2 * D, D)], _S_WV)
    c_wo = cp(wo_hbm, wo_s, _S_WO)
    c_w1 = cp(w1_hbm, w1_s, _S_W1)
    c_w2 = cp(w2_hbm, w2_s, _S_W2)
    c_b1 = cp(b1_hbm, b1_s, _S_B1)
    c_b2 = cp(b2_hbm, b2_s, _S_B2)

    def ln_rows(j):
        return _layernorm(x_s[pl.ds(_aligned(j, TS1), TS1), :].astype(f32)).astype(bf16)

    def softmax_group(pT, r0):
        p = pT[r0:r0 + 128, :].reshape(DH, 8, TS1)
        mx = jnp.max(p, axis=0, keepdims=True)
        mn = jnp.min(p, axis=0, keepdims=True)
        ep = jnp.exp(p - mx)
        en = jnp.exp(mn - p)
        sp = jnp.sum(ep, axis=0, keepdims=True)
        sn = jnp.sum(en, axis=0, keepdims=True)
        pp = (ep * (1.0 / sp)).reshape(128, TS1)
        pn = (en * (1.0 / sn)).reshape(128, TS1)
        return jnp.concatenate([pp, pn], axis=0)

    def feat_q(j, pTq):
        for g in range(G):
            phi = softmax_group(pTq, g * 128)
            phiq_s[g * 256:(g + 1) * 256, pl.ds(_aligned(j, TS1), TS1)] = phi.astype(bf16)

    def feat_k(pTk, xn, init=False):
        v = _dot(xn, wqkv_s[:, 2 * D:3 * D]).astype(bf16)
        for g in range(G):
            phi = softmax_group(pTk, g * 128)
            kv = _dot(phi.astype(bf16), v[:, g * 128:(g + 1) * 128])
            zz = phi[:, 0:128]
            for c in range(1, TS1 // 128):
                zz = zz + phi[:, c * 128:(c + 1) * 128]
            if init:
                kv_s[g] = kv
                z_s[g] = zz
            else:
                kv_s[g] += kv
                z_s[g] += zz

    def subtile(j, xn):
        pT = _dot_nt(wqkT_s[...], xn)
        feat_q(j, pT[0:D])
        feat_k(pT[D:2 * D], xn)

    c_wphi.start()
    x_copy(0).start()
    c_wq.start()
    c_wk.start()
    x_copy(1).start()

    c_wphi.wait()
    a = wphi_s[...].reshape(DH * DH, H)
    sel = jnp.where(_iota((H, D), 0) == _iota((H, D), 1) // DH, 1.0, 0.0).astype(bf16)
    b = _dot(a, sel)
    b = jnp.where(_iota((256, D), 0) // DH == _iota((256, D), 1) % DH, b, 0.0).astype(bf16)
    r = jnp.where(_iota((128, 256), 0) // 8 == _iota((128, 256), 1) % DH, 1.0, 0.0).astype(bf16)
    p = _dot(r, b)
    p = jnp.where(_iota((128, D), 0) % 8 == (_iota((128, D), 1) // DH) % 8, p, 0.0).astype(bf16)

    x_copy(0).wait()
    xn0 = ln_rows(0)

    def fold(qk):
        ws = []
        for g in range(G):
            c = qk * G + g
            w = wqkv_s[:, c * 128:(c + 1) * 128]
            ws.append(_dot_nt(p[:, g * 128:(g + 1) * 128], w).astype(bf16))
        wh = jnp.concatenate(ws, axis=0)
        wqkT_s[qk * D:(qk + 1) * D, :] = wh
        return wh

    c_wq.wait()
    c_wv.start()
    pTq0 = _dot_nt(fold(0), xn0)
    c_wk.wait()
    x_copy(1).wait()
    x_copy(2).start()
    pTk0 = _dot_nt(fold(1), xn0)
    feat_q(0, pTq0)
    xn1 = ln_rows(1)

    c_wv.wait()
    x_copy(2).wait()
    for c in range(3, NXC):
        x_copy(c).start()
    c_wo.start()
    c_b1.start()
    c_b2.start()
    c_w1.start()
    c_w2.start()
    feat_k(pTk0, xn0, init=True)
    subtile(1, xn1)
    xn_s[...] = ln_rows(2)

    def phase1(k, carry):
        j0 = 2 + k * NSI
        for s in range(1, NSI):
            x_copy(j0 + s).wait()

        @pl.when(j0 + NSI < NXC)
        def _():
            x_copy(j0 + NSI).wait()

        xns = [xn_s[...]] + [ln_rows(j0 + s) for s in range(1, NSI)]
        for s in range(NSI):
            subtile(j0 + s, xns[s])
        xn_s[...] = ln_rows(jnp.minimum(j0 + NSI, NXC - 1))
        return carry

    lax.fori_loop(0, NIT, phase1, 0)

    c_wo.wait()
    c_b1.wait()
    c_b2.wait()
    c_w1.wait()
    c_w2.wait()
    eye = jnp.where(_iota((128, 128), 0) == _iota((128, 128), 1), 1.0, 0.0).astype(bf16)
    kmask = (_iota((128, 256), 0) // DH) == (_iota((128, 256), 1) % 8)
    for g in range(G):
        kvT = _dot_nt(eye, kv_s[g].astype(bf16))
        kvT_s[g] = jnp.where(kmask, kvT, 0.0).astype(bf16)
        z_s[g] = jnp.broadcast_to(jnp.sum(z_s[g], axis=1, keepdims=True), (256, 128))

    def phase2(t, carry):
        b1 = b1_s[...].reshape(1, F).astype(f32)
        b2 = b2_s[...].reshape(1, D).astype(f32)
        hs = []
        hns = []
        for s in range(NS2):
            rows = pl.ds(_aligned(t * NS2 + s, TS2), TS2)
            x = x_s[rows, :].astype(f32)
            oTs = []
            for g in range(G):
                ph = phiq_s[g * 256:(g + 1) * 256, rows]
                nd = _dot(kvT_s[g], ph)
                phf = ph.astype(f32).reshape(2 * DH, 8, TS2)
                zb = z_s[g].reshape(2 * DH, 8, 128)
                den = jnp.concatenate(
                    [jnp.sum(phf[:, :, c * 128:(c + 1) * 128] * zb, axis=0)
                     for c in range(TS2 // 128)], axis=1)
                rcp = 1.0 / (den + DEN_EPS)
                for j in range(8):
                    oTs.append(nd[j * DH:(j + 1) * DH, :] * rcp[j:j + 1, :])
            oT = jnp.concatenate(oTs, axis=0)
            o = oT.T.astype(bf16)
            h = x + _dot(o, wo_s[...])
            hs.append(h)
            hns.append(_layernorm(h).astype(bf16))
        nc = F // FC
        npc = TS2 // TO
        for s in range(NS2):
            hn = hns[s]
            acc = hs[s] + b2
            for c in range(nc):
                h1 = _dot(hn, w1_s[:, c * FC:(c + 1) * FC])
                h1 = h1 + b1[:, c * FC:(c + 1) * FC]
                h1 = jnp.maximum(h1, 0.0)
                h1 = (h1 * h1).astype(bf16)
                if c < nc - 1:
                    acc = acc + _dot(h1, w2_s[c * FC:(c + 1) * FC, :])
                else:
                    for u in range(npc):
                        oc = (t * NS2 + s) * npc + u
                        orow = pl.ds(_aligned(oc, TO), TO)
                        if u < npc - 1:
                            part = acc[u * TO:(u + 1) * TO, :] + _dot(
                                h1[u * TO:(u + 1) * TO, :], w2_s[c * FC:(c + 1) * FC, :])
                            out_s[orow, :] = part.astype(bf16)
                            for w in range(NCS):
                                o_copy(oc, w).start()
                        else:
                            for w in range(NCS):
                                part = acc[u * TO:(u + 1) * TO, w * CW:(w + 1) * CW] + _dot(
                                    h1[u * TO:(u + 1) * TO, :], w2_s[c * FC:(c + 1) * FC, w * CW:(w + 1) * CW])
                                out_s[orow, w * CW:(w + 1) * CW] = part.astype(bf16)
                                o_copy(oc, w).start()
        return carry

    lax.fori_loop(0, N2, phase2, 0)

    for c in range(NOC):
        for w in range(NCS):
            o_copy(c, w).wait()


@jax.jit
def pallas_sequential_preLN__linear_kernel_hedgehog__dense_activation_squared_relu__prompt_kernel(
    A_x: jax.Array,
    A_wqkv: jax.Array,
    A_w_phi: jax.Array,
    A_wo: jax.Array,
    B_x: jax.Array,
    B_w1: jax.Array,
    B_b1: jax.Array,
    B_w2: jax.Array,
    B_b2: jax.Array,
):
    del B_x
    wphi_t = A_w_phi.transpose(1, 2, 0)

    any_spec = pl.BlockSpec(memory_space=pl.ANY)
    return pl.pallas_call(
        _kernel,
        in_specs=[any_spec] * 8,
        out_specs=any_spec,
        scratch_shapes=[
            pltpu.VMEM((S, D), bf16),
            pltpu.VMEM((D, 3 * D), bf16),
            pltpu.VMEM((DH, DH, H), bf16),
            pltpu.VMEM((F,), bf16),
            pltpu.VMEM((D,), bf16),
            pltpu.VMEM((2 * D, D), bf16),
            pltpu.VMEM((D, D), bf16),
            pltpu.VMEM((D, F), bf16),
            pltpu.VMEM((F, D), bf16),
            pltpu.VMEM((TS1, D), bf16),
            pltpu.VMEM((2 * D, S), bf16),
            pltpu.VMEM((G, 256, 128), f32),
            pltpu.VMEM((G, 256, 128), f32),
            pltpu.VMEM((G, 128, 256), bf16),
            pltpu.VMEM((S, D), bf16),
            pltpu.SemaphoreType.DMA((_NSEM,)),
        ],
        out_shape=jax.ShapeDtypeStruct((1, S, D), bf16),
        compiler_params=pltpu.CompilerParams(
            vmem_limit_bytes=100 * 1024 * 1024,
        ),
    )(A_x, A_wqkv, wphi_t, B_b1, B_b2, A_wo, B_w1, B_w2)
```

```python
import jax
import jax.numpy as jnp
import jax.experimental.pallas as pl
import jax.experimental.pallas.tpu as pltpu
from jax import lax

S, D, H, DH, F = 2048, 512, 32, 16, 1792
G = D // 128
TS1 = 256
NXC = S // TS1
NSI = 3
NIT = (NXC - 2) // NSI
TS2 = 512
NS2 = 2
N2 = S // (TS2 * NS2)
TO = 256
NOC = S // TO
NCS = 2
CW = D // NCS
FC = 896
LN_EPS = 1e-5
DEN_EPS = 1e-6

_NT_DIMS = (((1,), (1,)), ((), ()))
bf16 = jnp.bfloat16
f32 = jnp.float32

_S_WPHI, _S_WQ, _S_WK, _S_WV, _S_WO, _S_W1, _S_W2, _S_B1, _S_B2 = range(9)
_S_X = 9
_S_O = _S_X + NXC
_NSEM = _S_O + NOC * NCS


def _dot(a, b):
    return jnp.dot(a, b, preferred_element_type=f32)


def _dot_nt(a, b):
    return lax.dot_general(a, b, _NT_DIMS, preferred_element_type=f32)


def _layernorm(x):
    m = jnp.mean(x, axis=-1, keepdims=True)
    xc = x - m
    v = jnp.mean(xc * xc, axis=-1, keepdims=True)
    return xc * lax.rsqrt(v + LN_EPS)


def _iota(shape, dim):
    return lax.broadcasted_iota(jnp.int32, shape, dim)


def _aligned(c, n):
    return c * n if isinstance(c, int) else pl.multiple_of(c * n, n)


def _kernel(x_hbm, wqkv_hbm, wphi_hbm, b1_hbm, b2_hbm, wo_hbm, w1_hbm, w2_hbm,
            o_hbm,
            x_s, wqkv_s, wphi_s, b1_s, b2_s, wqkT_s, wo_s, w1_s, w2_s,
            xn_s, phiq_s, kv_s, z_s, kvT_s, out_s, sems):

    def cp(src, dst, k):
        return pltpu.make_async_copy(src, dst, sems.at[k])

    def x_copy(c):
        start = _aligned(c, TS1)
        return cp(x_hbm.at[0, pl.ds(start, TS1), :], x_s.at[pl.ds(start, TS1), :], _S_X + c)

    def o_copy(c, w):
        start = _aligned(c, TO)
        return cp(out_s.at[pl.ds(start, TO), pl.ds(w * CW, CW)],
                  o_hbm.at[0, pl.ds(start, TO), pl.ds(w * CW, CW)], _S_O + c * NCS + w)

    c_wphi = cp(wphi_hbm, wphi_s, _S_WPHI)
    c_wq = cp(wqkv_hbm.at[:, pl.ds(0, D)], wqkv_s.at[:, pl.ds(0, D)], _S_WQ)
    c_wk = cp(wqkv_hbm.at[:, pl.ds(D, D)], wqkv_s.at[:, pl.ds(D, D)], _S_WK)
    c_wv = cp(wqkv_hbm.at[:, pl.ds(2 * D, D)], wqkv_s.at[:, pl.ds(2 * D, D)], _S_WV)
    c_wo = cp(wo_hbm, wo_s, _S_WO)
    c_w1 = cp(w1_hbm, w1_s, _S_W1)
    c_w2 = cp(w2_hbm, w2_s, _S_W2)
    c_b1 = cp(b1_hbm, b1_s, _S_B1)
    c_b2 = cp(b2_hbm, b2_s, _S_B2)

    def ln_rows(j):
        return _layernorm(x_s[pl.ds(_aligned(j, TS1), TS1), :].astype(f32)).astype(bf16)

    def softmax_group(pT, r0):
        outs = []
        for u in range(2):
            p = pT[r0 + u * 64:r0 + (u + 1) * 64, :].reshape(8, 8, TS1)
            mx = jnp.max(p, axis=0)
            mx = jnp.maximum(mx, pltpu.roll(mx, 4, 0))
            mn = jnp.min(p, axis=0)
            mn = jnp.minimum(mn, pltpu.roll(mn, 4, 0))
            ep = jnp.exp(p - mx[None])
            en = jnp.exp(mn[None] - p)
            sp = jnp.sum(ep, axis=0)
            sp = sp + pltpu.roll(sp, 4, 0)
            sn = jnp.sum(en, axis=0)
            sn = sn + pltpu.roll(sn, 4, 0)
            outs.append((ep * (1.0 / sp)[None]).reshape(64, TS1))
            outs.append((en * (1.0 / sn)[None]).reshape(64, TS1))
        return jnp.concatenate(outs, axis=0)

    def feat_q(j, pTq):
        for g in range(G):
            phi = softmax_group(pTq, g * 128)
            phiq_s[g * 256:(g + 1) * 256, pl.ds(_aligned(j, TS1), TS1)] = phi.astype(bf16)

    def feat_k(pTk, vT, init=False):
        vTb = vT.astype(bf16)
        for g in range(G):
            phi = softmax_group(pTk, g * 128)
            phib = phi.astype(bf16)
            zz = phi[:, 0:128]
            for c in range(1, TS1 // 128):
                zz = zz + phi[:, c * 128:(c + 1) * 128]
            for u in range(2):
                gu = 2 * g + u
                kv = _dot_nt(vTb[gu * 64:(gu + 1) * 64, :], phib[u * 128:(u + 1) * 128, :])
                if init:
                    kv_s[gu] = kv
                else:
                    kv_s[gu] += kv
            if init:
                z_s[g] = zz
            else:
                z_s[g] += zz

    def subtile(j, xn):
        pT = _dot_nt(wqkT_s[...], xn)
        feat_q(j, pT[0:D])
        feat_k(pT[D:2 * D], pT[2 * D:3 * D])

    c_wphi.start()
    x_copy(0).start()
    c_wq.start()
    c_wk.start()
    x_copy(1).start()

    c_wphi.wait()
    a = wphi_s[...].reshape(DH * DH, H)
    sel = jnp.where(_iota((H, D), 0) == _iota((H, D), 1) // DH, 1.0, 0.0).astype(bf16)
    b = _dot(a, sel)
    b = jnp.where(_iota((256, D), 0) // DH == _iota((256, D), 1) % DH, b, 0.0).astype(bf16)
    rr = _iota((128, 256), 0)
    frow = 2 * ((rr % 64) // 8) + (rr % 8) // 4
    r = jnp.where(frow == _iota((128, 256), 1) % DH, 1.0, 0.0).astype(bf16)
    p = _dot(r, b)
    rr = _iota((128, D), 0)
    jrow = 4 * (rr // 64) + rr % 4
    p = jnp.where(jrow == (_iota((128, D), 1) // DH) % 8, p, 0.0).astype(bf16)

    x_copy(0).wait()
    xn0 = ln_rows(0)

    def fold(qk):
        ws = []
        for g in range(G):
            c = qk * G + g
            w = wqkv_s[:, c * 128:(c + 1) * 128]
            ws.append(_dot_nt(p[:, g * 128:(g + 1) * 128], w).astype(bf16))
        wh = jnp.concatenate(ws, axis=0)
        wqkT_s[qk * D:(qk + 1) * D, :] = wh
        return wh

    c_wq.wait()
    c_wv.start()
    pTq0 = _dot_nt(fold(0), xn0)
    c_wk.wait()
    x_copy(1).wait()
    x_copy(2).start()
    pTk0 = _dot_nt(fold(1), xn0)
    feat_q(0, pTq0)
    xn1 = ln_rows(1)

    c_wv.wait()
    x_copy(2).wait()
    for c in range(3, NXC):
        x_copy(c).start()
    c_wo.start()
    c_b1.start()
    c_b2.start()
    c_w1.start()
    c_w2.start()
    eye = jnp.where(_iota((128, 128), 0) == _iota((128, 128), 1), 1.0, 0.0).astype(bf16)
    wvT = jnp.concatenate(
        [_dot_nt(eye, wqkv_s[:, 2 * D + g * 128:2 * D + (g + 1) * 128]).astype(bf16)
         for g in range(G)], axis=0)
    wqkT_s[2 * D:3 * D, :] = wvT
    feat_k(pTk0, _dot_nt(wvT, xn0), init=True)
    subtile(1, xn1)
    xn_s[...] = ln_rows(2)

    def phase1(k, carry):
        j0 = 2 + k * NSI
        for s in range(1, NSI):
            x_copy(j0 + s).wait()

        @pl.when(j0 + NSI < NXC)
        def _():
            x_copy(j0 + NSI).wait()

        xns = [xn_s[...]] + [ln_rows(j0 + s) for s in range(1, NSI)]
        for s in range(NSI):
            subtile(j0 + s, xns[s])
        xn_s[...] = ln_rows(jnp.minimum(j0 + NSI, NXC - 1))
        return carry

    lax.fori_loop(0, NIT, phase1, 0)

    c_wo.wait()
    c_b1.wait()
    c_b2.wait()
    c_w1.wait()
    c_w2.wait()
    kmask = (_iota((64, 128), 0) // DH) == (_iota((64, 128), 1) % 4)
    for gu in range(2 * G):
        kvT_s[gu] = jnp.where(kmask, kv_s[gu], 0.0).astype(bf16)
    for g in range(G):
        z_s[g] = jnp.broadcast_to(jnp.sum(z_s[g], axis=1, keepdims=True), (256, 128))

    def phase2(t, carry):
        b1 = b1_s[...].reshape(1, F).astype(f32)
        b2 = b2_s[...].reshape(1, D).astype(f32)
        hs = []
        hns = []
        for s in range(NS2):
            rows = pl.ds(_aligned(t * NS2 + s, TS2), TS2)
            x = x_s[rows, :].astype(f32)
            oTs = []
            for gu in range(2 * G):
                ph = phiq_s[gu * 128:(gu + 1) * 128, rows]
                nd = _dot(kvT_s[gu], ph)
                phf = ph.astype(f32).reshape(DH, 8, TS2)
                zb = z_s[gu // 2, (gu % 2) * 128:(gu % 2 + 1) * 128, :].reshape(DH, 8, 128)
                den = jnp.concatenate(
                    [jnp.sum(phf[:, :, c * 128:(c + 1) * 128] * zb, axis=0)
                     for c in range(TS2 // 128)], axis=1)
                den = den + pltpu.roll(den, 4, 0)
                rcp = 1.0 / (den + DEN_EPS)
                for j in range(4):
                    oTs.append(nd[j * DH:(j + 1) * DH, :] * rcp[j:j + 1, :])
            oT = jnp.concatenate(oTs, axis=0)
            o = oT.T.astype(bf16)
            h = x + _dot(o, wo_s[...])
            hs.append(h)
            hns.append(_layernorm(h).astype(bf16))
        nc = F // FC
        npc = TS2 // TO
        for s in range(NS2):
            hn = hns[s]
            acc = hs[s] + b2
            for c in range(nc):
                h1 = _dot(hn, w1_s[:, c * FC:(c + 1) * FC])
                h1 = h1 + b1[:, c * FC:(c + 1) * FC]
                h1 = jnp.maximum(h1, 0.0)
                h1 = (h1 * h1).astype(bf16)
                if c < nc - 1:
                    acc = acc + _dot(h1, w2_s[c * FC:(c + 1) * FC, :])
                else:
                    for u in range(npc):
                        oc = (t * NS2 + s) * npc + u
                        orow = pl.ds(_aligned(oc, TO), TO)
                        if u < npc - 1:
                            part = acc[u * TO:(u + 1) * TO, :] + _dot(
                                h1[u * TO:(u + 1) * TO, :], w2_s[c * FC:(c + 1) * FC, :])
                            out_s[orow, :] = part.astype(bf16)
                            for w in range(NCS):
                                o_copy(oc, w).start()
                        else:
                            for w in range(NCS):
                                part = acc[u * TO:(u + 1) * TO, w * CW:(w + 1) * CW] + _dot(
                                    h1[u * TO:(u + 1) * TO, :], w2_s[c * FC:(c + 1) * FC, w * CW:(w + 1) * CW])
                                out_s[orow, w * CW:(w + 1) * CW] = part.astype(bf16)
                                o_copy(oc, w).start()
        return carry

    lax.fori_loop(0, N2, phase2, 0)

    for c in range(NOC):
        for w in range(NCS):
            o_copy(c, w).wait()


@jax.jit
def pallas_sequential_preLN__linear_kernel_hedgehog__dense_activation_squared_relu__prompt_kernel(
    A_x: jax.Array,
    A_wqkv: jax.Array,
    A_w_phi: jax.Array,
    A_wo: jax.Array,
    B_x: jax.Array,
    B_w1: jax.Array,
    B_b1: jax.Array,
    B_w2: jax.Array,
    B_b2: jax.Array,
):
    del B_x
    wphi_t = A_w_phi.transpose(1, 2, 0)

    any_spec = pl.BlockSpec(memory_space=pl.ANY)
    return pl.pallas_call(
        _kernel,
        in_specs=[any_spec] * 8,
        out_specs=any_spec,
        scratch_shapes=[
            pltpu.VMEM((S, D), bf16),
            pltpu.VMEM((D, 3 * D), bf16),
            pltpu.VMEM((DH, DH, H), bf16),
            pltpu.VMEM((F,), bf16),
            pltpu.VMEM((D,), bf16),
            pltpu.VMEM((3 * D, D), bf16),
            pltpu.VMEM((D, D), bf16),
            pltpu.VMEM((D, F), bf16),
            pltpu.VMEM((F, D), bf16),
            pltpu.VMEM((TS1, D), bf16),
            pltpu.VMEM((2 * D, S), bf16),
            pltpu.VMEM((2 * G, 64, 128), f32),
            pltpu.VMEM((G, 256, 128), f32),
            pltpu.VMEM((2 * G, 64, 128), bf16),
            pltpu.VMEM((S, D), bf16),
            pltpu.SemaphoreType.DMA((_NSEM,)),
        ],
        out_shape=jax.ShapeDtypeStruct((1, S, D), bf16),
        compiler_params=pltpu.CompilerParams(
            vmem_limit_bytes=100 * 1024 * 1024,
        ),
    )(A_x, A_wqkv, wphi_t, B_b1, B_b2, A_wo, B_w1, B_w2)
```

```python
import jax
import jax.numpy as jnp
import jax.experimental.pallas as pl
import jax.experimental.pallas.tpu as pltpu
from jax import lax

S, D, H, DH, F = 2048, 512, 32, 16, 1792
G = D // 128
TS1 = 256
NXC = S // TS1
TS2 = 512
NS2 = 2
N2 = S // (TS2 * NS2)
TO = 256
NOC = S // TO
NCS = 2
CW = D // NCS
FC = 896
LN_EPS = 1e-5
DEN_EPS = 1e-6

_NT_DIMS = (((1,), (1,)), ((), ()))
bf16 = jnp.bfloat16
f32 = jnp.float32

_S_WPHI, _S_WQ, _S_WK, _S_WV, _S_WO, _S_W1, _S_W2, _S_B1, _S_B2 = range(9)
_S_X = 9
_S_O = _S_X + NXC
_NSEM = _S_O + NOC * NCS


def _dot(a, b):
    return jnp.dot(a, b, preferred_element_type=f32)


def _dot_nt(a, b):
    return lax.dot_general(a, b, _NT_DIMS, preferred_element_type=f32)


def _layernorm(x):
    m = jnp.mean(x, axis=-1, keepdims=True)
    xc = x - m
    v = jnp.mean(xc * xc, axis=-1, keepdims=True)
    return xc * lax.rsqrt(v + LN_EPS)


def _iota(shape, dim):
    return lax.broadcasted_iota(jnp.int32, shape, dim)


def _aligned(c, n):
    return c * n if isinstance(c, int) else pl.multiple_of(c * n, n)


def _kernel(x_hbm, wqkv_hbm, wphi_hbm, b1_hbm, b2_hbm, wo_hbm, w1_hbm, w2_hbm,
            o_hbm,
            x_s, wqkv_s, wphi_s, b1_s, b2_s, wqkT_s, wo_s, w1_s, w2_s,
            phiq_s, kv_s, z_s, kvT_s, out_s, sems):

    def cp(src, dst, k):
        return pltpu.make_async_copy(src, dst, sems.at[k])

    def x_copy(c):
        start = _aligned(c, TS1)
        return cp(x_hbm.at[0, pl.ds(start, TS1), :], x_s.at[pl.ds(start, TS1), :], _S_X + c)

    def o_copy(c, w):
        start = _aligned(c, TO)
        return cp(out_s.at[pl.ds(start, TO), pl.ds(w * CW, CW)],
                  o_hbm.at[0, pl.ds(start, TO), pl.ds(w * CW, CW)], _S_O + c * NCS + w)

    c_wphi = cp(wphi_hbm, wphi_s, _S_WPHI)
    c_wq = cp(wqkv_hbm.at[:, pl.ds(0, D)], wqkv_s.at[:, pl.ds(0, D)], _S_WQ)
    c_wk = cp(wqkv_hbm.at[:, pl.ds(D, D)], wqkv_s.at[:, pl.ds(D, D)], _S_WK)
    c_wv = cp(wqkv_hbm.at[:, pl.ds(2 * D, D)], wqkv_s.at[:, pl.ds(2 * D, D)], _S_WV)
    c_wo = cp(wo_hbm, wo_s, _S_WO)
    c_w1 = cp(w1_hbm, w1_s, _S_W1)
    c_w2 = cp(w2_hbm, w2_s, _S_W2)
    c_b1 = cp(b1_hbm, b1_s, _S_B1)
    c_b2 = cp(b2_hbm, b2_s, _S_B2)

    def ln_rows(j):
        return _layernorm(x_s[pl.ds(_aligned(j, TS1), TS1), :].astype(f32)).astype(bf16)

    def softmax_group(pT, r0):
        outs = []
        for u in range(2):
            p = pT[r0 + u * 64:r0 + (u + 1) * 64, :].reshape(8, 8, TS1)
            mx = jnp.max(p, axis=0)
            mx = jnp.maximum(mx, pltpu.roll(mx, 4, 0))
            mn = jnp.min(p, axis=0)
            mn = jnp.minimum(mn, pltpu.roll(mn, 4, 0))
            ep = jnp.exp(p - mx[None])
            en = jnp.exp(mn[None] - p)
            sp = jnp.sum(ep, axis=0)
            sp = sp + pltpu.roll(sp, 4, 0)
            sn = jnp.sum(en, axis=0)
            sn = sn + pltpu.roll(sn, 4, 0)
            outs.append((ep * (1.0 / sp)[None]).reshape(64, TS1))
            outs.append((en * (1.0 / sn)[None]).reshape(64, TS1))
        return jnp.concatenate(outs, axis=0)

    def feat_q(j, pTq):
        for g in range(G):
            phi = softmax_group(pTq, g * 128)
            phiq_s[g * 256:(g + 1) * 256, pl.ds(_aligned(j, TS1), TS1)] = phi.astype(bf16)

    def feat_k(pTk, vT, init=False):
        vTb = vT.astype(bf16)
        for g in range(G):
            phi = softmax_group(pTk, g * 128)
            phib = phi.astype(bf16)
            zz = phi[:, 0:128]
            for c in range(1, TS1 // 128):
                zz = zz + phi[:, c * 128:(c + 1) * 128]
            for u in range(2):
                gu = 2 * g + u
                kv = _dot_nt(vTb[gu * 64:(gu + 1) * 64, :], phib[u * 128:(u + 1) * 128, :])
                if init:
                    kv_s[gu] = kv
                else:
                    kv_s[gu] += kv
            if init:
                z_s[g] = zz
            else:
                z_s[g] += zz

    def subtile(j, xn):
        pT = _dot_nt(wqkT_s[...], xn)
        feat_q(j, pT[0:D])
        feat_k(pT[D:2 * D], pT[2 * D:3 * D])

    c_wphi.start()
    x_copy(0).start()
    c_wq.start()
    c_wk.start()
    x_copy(1).start()

    c_wphi.wait()
    a = wphi_s[...].reshape(DH * DH, H)
    sel = jnp.where(_iota((H, D), 0) == _iota((H, D), 1) // DH, 1.0, 0.0).astype(bf16)
    b = _dot(a, sel)
    b = jnp.where(_iota((256, D), 0) // DH == _iota((256, D), 1) % DH, b, 0.0).astype(bf16)
    rr = _iota((128, 256), 0)
    frow = 2 * ((rr % 64) // 8) + (rr % 8) // 4
    r = jnp.where(frow == _iota((128, 256), 1) % DH, 1.0, 0.0).astype(bf16)
    p = _dot(r, b)
    rr = _iota((128, D), 0)
    jrow = 4 * (rr // 64) + rr % 4
    p = jnp.where(jrow == (_iota((128, D), 1) // DH) % 8, p, 0.0).astype(bf16)

    x_copy(0).wait()
    xn0 = ln_rows(0)

    def fold(qk):
        ws = []
        for g in range(G):
            c = qk * G + g
            w = wqkv_s[:, c * 128:(c + 1) * 128]
            ws.append(_dot_nt(p[:, g * 128:(g + 1) * 128], w).astype(bf16))
        wh = jnp.concatenate(ws, axis=0)
        wqkT_s[qk * D:(qk + 1) * D, :] = wh
        return wh

    c_wq.wait()
    c_wv.start()
    pTq0 = _dot_nt(fold(0), xn0)
    c_wk.wait()
    x_copy(1).wait()
    x_copy(2).start()
    pTk0 = _dot_nt(fold(1), xn0)
    feat_q(0, pTq0)
    xn1 = ln_rows(1)

    c_wv.wait()
    x_copy(2).wait()
    for c in range(3, NXC):
        x_copy(c).start()
    c_wo.start()
    c_b1.start()
    c_b2.start()
    c_w1.start()
    c_w2.start()
    eye = jnp.where(_iota((128, 128), 0) == _iota((128, 128), 1), 1.0, 0.0).astype(bf16)
    wvT = jnp.concatenate(
        [_dot_nt(eye, wqkv_s[:, 2 * D + g * 128:2 * D + (g + 1) * 128]).astype(bf16)
         for g in range(G)], axis=0)
    wqkT_s[2 * D:3 * D, :] = wvT
    feat_k(pTk0, _dot_nt(wvT, xn0), init=True)
    subtile(1, xn1)
    xn_next = ln_rows(2)

    for j in range(3, NXC):
        x_copy(j).wait()
    xns = [xn_next] + [ln_rows(j) for j in range(3, NXC)]
    for j in range(2, NXC):
        subtile(j, xns[j - 2])

    kmask = (_iota((64, 128), 0) // DH) == (_iota((64, 128), 1) % 4)
    for gu in range(2 * G):
        kvT_s[gu] = jnp.where(kmask, kv_s[gu], 0.0).astype(bf16)
    for g in range(G):
        z_s[g] = jnp.broadcast_to(jnp.sum(z_s[g], axis=1, keepdims=True), (256, 128))

    c_wo.wait()
    c_b1.wait()
    c_b2.wait()
    c_w1.wait()
    c_w2.wait()

    def phase2(t, carry):
        b1 = b1_s[...].reshape(1, F).astype(f32)
        b2 = b2_s[...].reshape(1, D).astype(f32)
        hs = []
        hns = []
        for s in range(NS2):
            rows = pl.ds(_aligned(t * NS2 + s, TS2), TS2)
            x = x_s[rows, :].astype(f32)
            oTs = []
            for gu in range(2 * G):
                ph = phiq_s[gu * 128:(gu + 1) * 128, rows]
                nd = _dot(kvT_s[gu], ph)
                phf = ph.astype(f32).reshape(DH, 8, TS2)
                zb = z_s[gu // 2, (gu % 2) * 128:(gu % 2 + 1) * 128, :].reshape(DH, 8, 128)
                den = jnp.concatenate(
                    [jnp.sum(phf[:, :, c * 128:(c + 1) * 128] * zb, axis=0)
                     for c in range(TS2 // 128)], axis=1)
                den = den + pltpu.roll(den, 4, 0)
                rcp = 1.0 / (den + DEN_EPS)
                for j in range(4):
                    oTs.append(nd[j * DH:(j + 1) * DH, :] * rcp[j:j + 1, :])
            oT = jnp.concatenate(oTs, axis=0)
            o = oT.T.astype(bf16)
            h = x + _dot(o, wo_s[...])
            hs.append(h)
            hns.append(_layernorm(h).astype(bf16))
        nc = F // FC
        npc = TS2 // TO
        for s in range(NS2):
            hn = hns[s]
            acc = hs[s] + b2
            for c in range(nc):
                h1 = _dot(hn, w1_s[:, c * FC:(c + 1) * FC])
                h1 = h1 + b1[:, c * FC:(c + 1) * FC]
                h1 = jnp.maximum(h1, 0.0)
                h1 = (h1 * h1).astype(bf16)
                if c < nc - 1:
                    acc = acc + _dot(h1, w2_s[c * FC:(c + 1) * FC, :])
                else:
                    for u in range(npc):
                        oc = (t * NS2 + s) * npc + u
                        orow = pl.ds(_aligned(oc, TO), TO)
                        if u < npc - 1:
                            part = acc[u * TO:(u + 1) * TO, :] + _dot(
                                h1[u * TO:(u + 1) * TO, :], w2_s[c * FC:(c + 1) * FC, :])
                            out_s[orow, :] = part.astype(bf16)
                            for w in range(NCS):
                                o_copy(oc, w).start()
                        else:
                            for w in range(NCS):
                                part = acc[u * TO:(u + 1) * TO, w * CW:(w + 1) * CW] + _dot(
                                    h1[u * TO:(u + 1) * TO, :], w2_s[c * FC:(c + 1) * FC, w * CW:(w + 1) * CW])
                                out_s[orow, w * CW:(w + 1) * CW] = part.astype(bf16)
                                o_copy(oc, w).start()
        return carry

    lax.fori_loop(0, N2, phase2, 0)

    for c in range(NOC):
        for w in range(NCS):
            o_copy(c, w).wait()


@jax.jit
def pallas_sequential_preLN__linear_kernel_hedgehog__dense_activation_squared_relu__prompt_kernel(
    A_x: jax.Array,
    A_wqkv: jax.Array,
    A_w_phi: jax.Array,
    A_wo: jax.Array,
    B_x: jax.Array,
    B_w1: jax.Array,
    B_b1: jax.Array,
    B_w2: jax.Array,
    B_b2: jax.Array,
):
    del B_x
    wphi_t = A_w_phi.transpose(1, 2, 0)

    any_spec = pl.BlockSpec(memory_space=pl.ANY)
    return pl.pallas_call(
        _kernel,
        in_specs=[any_spec] * 8,
        out_specs=any_spec,
        scratch_shapes=[
            pltpu.VMEM((S, D), bf16),
            pltpu.VMEM((D, 3 * D), bf16),
            pltpu.VMEM((DH, DH, H), bf16),
            pltpu.VMEM((F,), bf16),
            pltpu.VMEM((D,), bf16),
            pltpu.VMEM((3 * D, D), bf16),
            pltpu.VMEM((D, D), bf16),
            pltpu.VMEM((D, F), bf16),
            pltpu.VMEM((F, D), bf16),
            pltpu.VMEM((2 * D, S), bf16),
            pltpu.VMEM((2 * G, 64, 128), f32),
            pltpu.VMEM((G, 256, 128), f32),
            pltpu.VMEM((2 * G, 64, 128), bf16),
            pltpu.VMEM((S, D), bf16),
            pltpu.SemaphoreType.DMA((_NSEM,)),
        ],
        out_shape=jax.ShapeDtypeStruct((1, S, D), bf16),
        compiler_params=pltpu.CompilerParams(
            vmem_limit_bytes=100 * 1024 * 1024,
        ),
    )(A_x, A_wqkv, wphi_t, B_b1, B_b2, A_wo, B_w1, B_w2)
```

```python
import jax
import jax.numpy as jnp
import jax.experimental.pallas as pl
import jax.experimental.pallas.tpu as pltpu
from jax import lax

S, D, H, DH, F = 2048, 512, 32, 16, 1792
G = D // 128
TS1 = 256
NXC = S // TS1
TS2 = 512
NS2 = 2
N2 = S // (TS2 * NS2)
TO = 256
NOC = S // TO
NCS = 2
CW = D // NCS
FC = 896
LN_EPS = 1e-5
DEN_EPS = 1e-6

_NT_DIMS = (((1,), (1,)), ((), ()))
bf16 = jnp.bfloat16
f32 = jnp.float32

_S_WPHI, _S_WQ, _S_WK, _S_WV, _S_WO, _S_W1, _S_W2, _S_B1, _S_B2 = range(9)
_S_X = 9
_S_O = _S_X + NXC
_NSEM = _S_O + NOC * NCS


def _dot(a, b):
    return jnp.dot(a, b, preferred_element_type=f32)


def _dot_nt(a, b):
    return lax.dot_general(a, b, _NT_DIMS, preferred_element_type=f32)


def _layernorm(x):
    m = jnp.mean(x, axis=-1, keepdims=True)
    xc = x - m
    v = jnp.mean(xc * xc, axis=-1, keepdims=True)
    return xc * lax.rsqrt(v + LN_EPS)


def _iota(shape, dim):
    return lax.broadcasted_iota(jnp.int32, shape, dim)


def _aligned(c, n):
    return c * n if isinstance(c, int) else pl.multiple_of(c * n, n)


def _kernel(x_hbm, wqkv_hbm, wphi_hbm, b1_hbm, b2_hbm, wo_hbm, w1_hbm, w2_hbm,
            o_hbm,
            x_s, wqkv_s, wphi_s, b1_s, b2_s, wqkT_s, wo_s, w1_s, w2_s,
            phiq_s, kv_s, z_s, kvT_s, out_s, sems):

    def cp(src, dst, k):
        return pltpu.make_async_copy(src, dst, sems.at[k])

    def x_copy(c):
        start = _aligned(c, TS1)
        return cp(x_hbm.at[0, pl.ds(start, TS1), :], x_s.at[pl.ds(start, TS1), :], _S_X + c)

    def o_copy(c, w):
        start = _aligned(c, TO)
        return cp(out_s.at[pl.ds(start, TO), pl.ds(w * CW, CW)],
                  o_hbm.at[0, pl.ds(start, TO), pl.ds(w * CW, CW)], _S_O + c * NCS + w)

    c_wphi = cp(wphi_hbm, wphi_s, _S_WPHI)
    c_wq = cp(wqkv_hbm.at[:, pl.ds(0, D)], wqkv_s.at[:, pl.ds(0, D)], _S_WQ)
    c_wk = cp(wqkv_hbm.at[:, pl.ds(D, D)], wqkv_s.at[:, pl.ds(D, D)], _S_WK)
    c_wv = cp(wqkv_hbm.at[:, pl.ds(2 * D, D)], wqkv_s.at[:, pl.ds(2 * D, D)], _S_WV)
    c_wo = cp(wo_hbm, wo_s, _S_WO)
    c_w1 = cp(w1_hbm, w1_s, _S_W1)
    c_w2 = cp(w2_hbm, w2_s, _S_W2)
    c_b1 = cp(b1_hbm, b1_s, _S_B1)
    c_b2 = cp(b2_hbm, b2_s, _S_B2)

    def ln_rows(j):
        return _layernorm(x_s[pl.ds(_aligned(j, TS1), TS1), :].astype(f32)).astype(bf16)

    def softmax_group(pT, r0):
        outs = []
        for u in range(2):
            p = pT[r0 + u * 64:r0 + (u + 1) * 64, :].reshape(8, 8, TS1)
            mx = jnp.max(p, axis=0)
            mx = jnp.maximum(mx, pltpu.roll(mx, 4, 0))
            mn = jnp.min(p, axis=0)
            mn = jnp.minimum(mn, pltpu.roll(mn, 4, 0))
            ep = jnp.exp(p - mx[None])
            en = jnp.exp(mn[None] - p)
            sp = jnp.sum(ep, axis=0)
            sp = sp + pltpu.roll(sp, 4, 0)
            sn = jnp.sum(en, axis=0)
            sn = sn + pltpu.roll(sn, 4, 0)
            outs.append((ep * (1.0 / sp)[None]).reshape(64, TS1))
            outs.append((en * (1.0 / sn)[None]).reshape(64, TS1))
        return jnp.concatenate(outs, axis=0)

    def feat_q(j, pTq):
        for g in range(G):
            phi = softmax_group(pTq, g * 128)
            phiq_s[g * 256:(g + 1) * 256, pl.ds(_aligned(j, TS1), TS1)] = phi.astype(bf16)

    def feat_k(pTk, vT, init=False, phis=None):
        vTb = vT.astype(bf16)
        for g in range(G):
            phi = softmax_group(pTk, g * 128) if phis is None else phis[g]
            phib = phi.astype(bf16)
            zz = phi[:, 0:128]
            for c in range(1, TS1 // 128):
                zz = zz + phi[:, c * 128:(c + 1) * 128]
            for u in range(2):
                gu = 2 * g + u
                kv = _dot_nt(vTb[gu * 64:(gu + 1) * 64, :], phib[u * 128:(u + 1) * 128, :])
                if init:
                    kv_s[gu] = kv
                else:
                    kv_s[gu] += kv
            if init:
                z_s[g] = zz
            else:
                z_s[g] += zz

    def subtile(j, xn):
        pT = _dot_nt(wqkT_s[...], xn)
        feat_q(j, pT[0:D])
        feat_k(pT[D:2 * D], pT[2 * D:3 * D])

    c_wphi.start()
    x_copy(0).start()
    c_wq.start()
    c_wk.start()
    x_copy(1).start()

    c_wphi.wait()
    a = wphi_s[...].reshape(DH * DH, H)
    sel = jnp.where(_iota((H, D), 0) == _iota((H, D), 1) // DH, 1.0, 0.0).astype(bf16)
    b = _dot(a, sel)
    b = jnp.where(_iota((256, D), 0) // DH == _iota((256, D), 1) % DH, b, 0.0).astype(bf16)
    rr = _iota((128, 256), 0)
    frow = 2 * ((rr % 64) // 8) + (rr % 8) // 4
    r = jnp.where(frow == _iota((128, 256), 1) % DH, 1.0, 0.0).astype(bf16)
    p = _dot(r, b)
    rr = _iota((128, D), 0)
    jrow = 4 * (rr // 64) + rr % 4
    p = jnp.where(jrow == (_iota((128, D), 1) // DH) % 8, p, 0.0).astype(bf16)

    x_copy(0).wait()
    xn0 = ln_rows(0)

    def fold(qk):
        ws = []
        for g in range(G):
            c = qk * G + g
            w = wqkv_s[:, c * 128:(c + 1) * 128]
            ws.append(_dot_nt(p[:, g * 128:(g + 1) * 128], w).astype(bf16))
        wh = jnp.concatenate(ws, axis=0)
        wqkT_s[qk * D:(qk + 1) * D, :] = wh
        return wh

    c_wq.wait()
    c_wv.start()
    pTq0 = _dot_nt(fold(0), xn0)
    c_wk.wait()
    x_copy(1).wait()
    x_copy(2).start()
    pTk0 = _dot_nt(fold(1), xn0)
    phik0 = [softmax_group(pTk0, g * 128) for g in range(G)]
    xn1 = ln_rows(1)

    c_wv.wait()
    x_copy(2).wait()
    for c in range(3, NXC):
        x_copy(c).start()
    c_wo.start()
    c_b1.start()
    c_b2.start()
    c_w1.start()
    c_w2.start()
    eye = jnp.where(_iota((128, 128), 0) == _iota((128, 128), 1), 1.0, 0.0).astype(bf16)
    wvT = jnp.concatenate(
        [_dot_nt(eye, wqkv_s[:, 2 * D + g * 128:2 * D + (g + 1) * 128]).astype(bf16)
         for g in range(G)], axis=0)
    wqkT_s[2 * D:3 * D, :] = wvT
    feat_k(None, _dot_nt(wvT, xn0), init=True, phis=phik0)
    feat_q(0, pTq0)
    subtile(1, xn1)
    xn_next = ln_rows(2)

    for j in range(3, NXC):
        x_copy(j).wait()
    xns = [xn_next] + [ln_rows(j) for j in range(3, NXC)]
    for j in range(2, NXC):
        subtile(j, xns[j - 2])

    kmask = (_iota((64, 128), 0) // DH) == (_iota((64, 128), 1) % 4)
    for gu in range(2 * G):
        kvT_s[gu] = jnp.where(kmask, kv_s[gu], 0.0).astype(bf16)
    for g in range(G):
        z_s[g] = jnp.broadcast_to(jnp.sum(z_s[g], axis=1, keepdims=True), (256, 128))

    c_wo.wait()
    c_b1.wait()
    c_b2.wait()
    c_w1.wait()
    c_w2.wait()

    def phase2(t, carry):
        b1 = b1_s[...].reshape(1, F).astype(f32)
        b2 = b2_s[...].reshape(1, D).astype(f32)
        hs = []
        hns = []
        for s in range(NS2):
            rows = pl.ds(_aligned(t * NS2 + s, TS2), TS2)
            x = x_s[rows, :].astype(f32)
            oTs = []
            for gu in range(2 * G):
                ph = phiq_s[gu * 128:(gu + 1) * 128, rows]
                nd = _dot(kvT_s[gu], ph)
                phf = ph.astype(f32).reshape(DH, 8, TS2)
                zb = z_s[gu // 2, (gu % 2) * 128:(gu % 2 + 1) * 128, :].reshape(DH, 8, 128)
                den = jnp.concatenate(
                    [jnp.sum(phf[:, :, c * 128:(c + 1) * 128] * zb, axis=0)
                     for c in range(TS2 // 128)], axis=1)
                den = den + pltpu.roll(den, 4, 0)
                rcp = 1.0 / (den + DEN_EPS)
                for j in range(4):
                    oTs.append(nd[j * DH:(j + 1) * DH, :] * rcp[j:j + 1, :])
            oT = jnp.concatenate(oTs, axis=0)
            o = oT.T.astype(bf16)
            h = x + _dot(o, wo_s[...])
            hs.append(h)
            hns.append(_layernorm(h).astype(bf16))
        nc = F // FC
        npc = TS2 // TO
        for s in range(NS2):
            hn = hns[s]
            acc = hs[s] + b2
            for c in range(nc):
                h1 = _dot(hn, w1_s[:, c * FC:(c + 1) * FC])
                h1 = h1 + b1[:, c * FC:(c + 1) * FC]
                h1 = jnp.maximum(h1, 0.0)
                h1 = (h1 * h1).astype(bf16)
                if c < nc - 1:
                    acc = acc + _dot(h1, w2_s[c * FC:(c + 1) * FC, :])
                else:
                    for u in range(npc):
                        oc = (t * NS2 + s) * npc + u
                        orow = pl.ds(_aligned(oc, TO), TO)
                        if u < npc - 1:
                            part = acc[u * TO:(u + 1) * TO, :] + _dot(
                                h1[u * TO:(u + 1) * TO, :], w2_s[c * FC:(c + 1) * FC, :])
                            out_s[orow, :] = part.astype(bf16)
                            for w in range(NCS):
                                o_copy(oc, w).start()
                        else:
                            for w in range(NCS):
                                part = acc[u * TO:(u + 1) * TO, w * CW:(w + 1) * CW] + _dot(
                                    h1[u * TO:(u + 1) * TO, :], w2_s[c * FC:(c + 1) * FC, w * CW:(w + 1) * CW])
                                out_s[orow, w * CW:(w + 1) * CW] = part.astype(bf16)
                                o_copy(oc, w).start()
        return carry

    lax.fori_loop(0, N2, phase2, 0)

    for c in range(NOC):
        for w in range(NCS):
            o_copy(c, w).wait()


@jax.jit
def pallas_sequential_preLN__linear_kernel_hedgehog__dense_activation_squared_relu__prompt_kernel(
    A_x: jax.Array,
    A_wqkv: jax.Array,
    A_w_phi: jax.Array,
    A_wo: jax.Array,
    B_x: jax.Array,
    B_w1: jax.Array,
    B_b1: jax.Array,
    B_w2: jax.Array,
    B_b2: jax.Array,
):
    del B_x
    wphi_t = A_w_phi.transpose(1, 2, 0)

    any_spec = pl.BlockSpec(memory_space=pl.ANY)
    return pl.pallas_call(
        _kernel,
        in_specs=[any_spec] * 8,
        out_specs=any_spec,
        scratch_shapes=[
            pltpu.VMEM((S, D), bf16),
            pltpu.VMEM((D, 3 * D), bf16),
            pltpu.VMEM((DH, DH, H), bf16),
            pltpu.VMEM((F,), bf16),
            pltpu.VMEM((D,), bf16),
            pltpu.VMEM((3 * D, D), bf16),
            pltpu.VMEM((D, D), bf16),
            pltpu.VMEM((D, F), bf16),
            pltpu.VMEM((F, D), bf16),
            pltpu.VMEM((2 * D, S), bf16),
            pltpu.VMEM((2 * G, 64, 128), f32),
            pltpu.VMEM((G, 256, 128), f32),
            pltpu.VMEM((2 * G, 64, 128), bf16),
            pltpu.VMEM((S, D), bf16),
            pltpu.SemaphoreType.DMA((_NSEM,)),
        ],
        out_shape=jax.ShapeDtypeStruct((1, S, D), bf16),
        compiler_params=pltpu.CompilerParams(
            vmem_limit_bytes=100 * 1024 * 1024,
        ),
    )(A_x, A_wqkv, wphi_t, B_b1, B_b2, A_wo, B_w1, B_w2)
```
